```python
import os as _os
_os.environ.setdefault("JAX_PLATFORMS", "cpu")
import jax
import jax.numpy as jnp

def _softmax(x, axis=-1):
    return jax.nn.softmax(x, axis=axis)
def _gelu(x):
    return jax.nn.gelu(x, approximate=True)
def _silu(x):
    return jax.nn.silu(x)
def _sigmoid(x):
    return jax.nn.sigmoid(x)
def _layernorm(x, axis=-1, eps=1e-5):
    m = jnp.mean(x, axis=axis, keepdims=True)
    v = jnp.var(x, axis=axis, keepdims=True)
    return (x - m) / jnp.sqrt(v + eps)
def _scatter_add(tgt, idx, src, axis=0):
    return tgt.at[idx].add(src)
def _segment_sum(src, seg, n):
    return jax.ops.segment_sum(src, seg, n)
class _Rng:
    def __init__(self, key):
        self._k = key
    def _next(self):
        self._k, sub = jax.random.split(self._k)
        return sub
    def normal(self, shape):
        return jax.random.normal(self._next(), shape, dtype=jnp.bfloat16)
    def randint(self, lo, hi, shape):
        return jax.random.randint(self._next(), shape, lo, hi, dtype=jnp.int32)
    def uniform(self, shape, lo=0.0, hi=1.0):
        return jax.random.uniform(self._next(), shape, jnp.bfloat16, lo, hi)
    def permutation(self, n):
        return jax.random.permutation(self._next(), n)


kernel_name = 'sequential_preLN__softmax_full_mha__glu_gated_swiglu__prompt'

def setup_inputs():
    _rng = _Rng(jax.random.key(int.from_bytes(__import__("os").urandom(4), "little")))
    _w = (lambda a: (lambda t: t.astype(jnp.bfloat16) if jnp.issubdtype(t.dtype, jnp.floating) else t)(jnp.asarray(a)))
    def _A_setup():
        B, S, D = 1, 2048, 640
        return {
            "x": _w((lambda *s: _rng.normal(s) * 0.05)(B, S, D)),
            "wqkv": _w((lambda *s: _rng.normal(s) * 0.05)(D, 3 * D)),
            "wo": _w((lambda *s: _rng.normal(s) * 0.05)(D, D)),
        }
    _A_in = _A_setup()

    def _B_setup():
        B, S, D, F = 1, 2048, 640, 1728
        return {
            "x": _w((lambda *s: _rng.normal(s) * 0.05)(B, S, D)),
            "w1": _w((lambda *s: _rng.normal(s) * 0.05)(D, F) * (2.0 / D) ** 0.5),
            "w3": _w((lambda *s: _rng.normal(s) * 0.05)(D, F) * (2.0 / D) ** 0.5),
            "w2": _w((lambda *s: _rng.normal(s) * 0.05)(F, D) * (2.0 / F) ** 0.5),
        }
    _B_in = _B_setup()

    return {
        "A_x": _A_in["x"],
        "A_wqkv": _A_in["wqkv"],
        "A_wo": _A_in["wo"],
        "B_x": _B_in["x"],
        "B_w1": _B_in["w1"],
        "B_w3": _B_in["w3"],
        "B_w2": _B_in["w2"],
    }

def reference(A_x, A_wqkv, A_wo, B_x, B_w1, B_w3, B_w2):
    def _A_ref(x, wqkv, wo):
        B, S, D = x.shape
        H = 32; Dh = D // H
        qkv = (lambda x, *d: x.transpose(*d))((x @ wqkv).reshape(B, S, 3, H, Dh), 2, 0, 3, 1, 4)
        q, k, v = qkv[0], qkv[1], qkv[2]
        scale = Dh ** -0.5
        scores = jnp.einsum("bhqd,bhkd->bhqk", q, k) * scale
        p = _softmax(scores, axis=-1)
        o = jnp.einsum("bhqk,bhkd->bhqd", p, v)
        return (lambda x, *d: x.transpose(*d))(o, 0, 2, 1, 3).reshape(B, S, D) @ wo

    def _B_ref(x, w1, w3, w2):
        gate = jnp.einsum("bsd,df->bsf", x, w1)
        up = jnp.einsum("bsd,df->bsf", x, w3)
        h = _silu(gate) * up
        out = jnp.einsum("bsf,fd->bsd", h, w2)
        return out

    x = A_x
    h = x + _A_ref(_layernorm(x, axis=-1), A_wqkv, A_wo)
    h2 = h + _B_ref(_layernorm(h, axis=-1), B_w1, B_w3, B_w2)
    return h2
```

```python
import functools, math
import jax, jax.numpy as jnp, numpy as np
from jax import lax
from jax.experimental import pallas as pl
from jax.experimental.pallas import tpu as pltpu

S, D, H, DH, F = 2048, 640, 32, 20, 1728
NT = 6
LOG2E = 1.4426950408889634
STRAD = (120, 240, 380, 500)

def _ln(x):
    m = jnp.mean(x, axis=-1, keepdims=True)
    xc = x - m
    v = jnp.mean(xc * xc, axis=-1, keepdims=True)
    return xc * lax.rsqrt(v + 1e-5)

def head_loc(h):
    lo = h * 20
    t = lo >> 7
    off = lo & 127
    st = off > 108
    sidx = (h > 6).astype(jnp.int32) + (h > 12).astype(jnp.int32) + (h > 19).astype(jnp.int32)
    return jnp.where(st, 5, t), jnp.where(st, 32 * sidx, off)

def make_kernel(MQ, HB=4, CH=512, FS=1):
    NQ = S // MQ
    def kernel(x_ref, wqkv_ref, wo_hbm, w1_hbm, w3_hbm, w2_hbm, o_ref, q_sc, k_sc, v_sc, o_sc, wox_sc, wo_ref, w1_ref, w3_ref, w2_ref, sems):
        i = pl.program_id(0)
        scale = (DH ** -0.5) * LOG2E
        lane = lax.broadcasted_iota(jnp.int32, (MQ, 128), 1)

        copies = [pltpu.make_async_copy(src, dst, sems.at[n]) for n, (src, dst) in enumerate(
            ((wo_hbm, wo_ref), (w1_hbm, w1_ref), (w3_hbm, w3_ref), (w2_hbm, w2_ref)))]

        @pl.when(i == 0)
        def _():
            for cp in copies:
                cp.start()
            def body(c, carry):
                c0 = pl.multiple_of(c * CH, CH)
                xc = x_ref[pl.ds(c0, CH), :].astype(jnp.float32)
                ln = _ln(xc).astype(jnp.bfloat16)
                qkv = jnp.dot(ln, wqkv_ref[...], preferred_element_type=jnp.float32)
                for (sc, base, mul) in ((q_sc, 0, scale), (k_sc, 640, None), (v_sc, 1280, None)):
                    part = qkv[:, base:base + 640]
                    if mul is not None:
                        part = part * mul
                    for t in range(5):
                        sc[t, pl.ds(c0, CH), :] = part[:, t * 128:(t + 1) * 128].astype(jnp.bfloat16)
                    pieces = []
                    for a in STRAD:
                        pieces.append(part[:, a:a + DH])
                        pieces.append(jnp.zeros((CH, 32 - DH), jnp.float32))
                    sc[5, pl.ds(c0, CH), :] = jnp.concatenate(pieces, axis=1).astype(jnp.bfloat16)
                return carry
            lax.fori_loop(0, S // CH, body, 0)
            copies[0].wait()
            pieces = []
            for a in STRAD:
                pieces.append(wo_ref[a:a + DH, :].astype(jnp.float32))
                pieces.append(jnp.zeros((32 - DH, D), jnp.float32))
            wox_sc[...] = jnp.concatenate(pieces, axis=0).astype(jnp.bfloat16)

        r0 = pl.multiple_of(i * MQ, MQ)
        o_sc[...] = jnp.zeros_like(o_sc)

        def body(j, carry):
            for t in range(HB):
                h = HB * j + t
                tile, off = head_loc(h)
                qg = q_sc[tile, pl.ds(r0, MQ), :]
                mask = (lane >= off) & (lane < off + DH)
                qm = jnp.where(mask, qg, jnp.zeros_like(qg))
                s = lax.dot_general(qm, k_sc[tile], (((1,), (1,)), ((), ())), preferred_element_type=jnp.float32)
                m = jnp.max(s, axis=-1, keepdims=True)
                p = jnp.exp2(s - m)
                l = jnp.sum(p, axis=-1, keepdims=True)
                o = jnp.dot(p.astype(jnp.bfloat16), v_sc[tile], preferred_element_type=jnp.float32)
                o_sc[tile] = jnp.where(mask, o / l, o_sc[tile])
            return carry
        lax.fori_loop(0, H // HB, body, 0)

        @pl.when(i == 0)
        def _():
            for cp in copies[1:]:
                cp.wait()

        FR = MQ // FS
        def ffn_body(c, carry):
            c0 = pl.multiple_of(c * FR, FR)
            attn = jnp.dot(o_sc[5, pl.ds(c0, FR), :].astype(jnp.bfloat16), wox_sc[...], preferred_element_type=jnp.float32)
            for t in range(5):
                attn = attn + jnp.dot(o_sc[t, pl.ds(c0, FR), :].astype(jnp.bfloat16), wo_ref[t * 128:(t + 1) * 128, :], preferred_element_type=jnp.float32)
            h = x_ref[pl.ds(r0 + c0, FR), :].astype(jnp.float32) + attn
            ln2 = _ln(h).astype(jnp.bfloat16)
            gate = lax.dot_general(ln2, w1_ref[...], (((1,), (1,)), ((), ())), preferred_element_type=jnp.float32)
            up = lax.dot_general(ln2, w3_ref[...], (((1,), (1,)), ((), ())), preferred_element_type=jnp.float32)
            hh = (gate * jax.nn.sigmoid(gate) * up).astype(jnp.bfloat16)
            out = h + jnp.dot(hh, w2_ref[...], preferred_element_type=jnp.float32)
            o_ref[pl.ds(c0, FR), :] = out.astype(o_ref.dtype)
            return carry
        lax.fori_loop(0, FS, ffn_body, 0)
    return kernel

@jax.jit
def pallas_sequential_preLN__softmax_full_mha__glu_gated_swiglu__prompt_kernel(A_x, A_wqkv, A_wo, B_x, B_w1, B_w3, B_w2):
    MQ, HB, CH, FS = 512, 8, 256, 2
    x = A_x.reshape(S, D)
    full = lambda shape: pl.BlockSpec(shape, lambda i: (0,) * len(shape))
    out = pl.pallas_call(
        make_kernel(MQ, HB, CH, FS),
        grid=(S // MQ,),
        in_specs=[full((S, D)), full((D, 3 * D))] + [pl.BlockSpec(memory_space=pl.ANY)] * 4,
        out_specs=pl.BlockSpec((MQ, D), lambda i: (i, 0)),
        out_shape=jax.ShapeDtypeStruct((S, D), jnp.bfloat16),
        scratch_shapes=[pltpu.VMEM((NT, S, 128), jnp.bfloat16), pltpu.VMEM((NT, S, 128), jnp.bfloat16),
                        pltpu.VMEM((NT, S, 128), jnp.bfloat16), pltpu.VMEM((NT, MQ, 128), jnp.float32),
                        pltpu.VMEM((128, D), jnp.bfloat16), pltpu.VMEM((D, D), jnp.bfloat16),
                        pltpu.VMEM((F, D), jnp.bfloat16), pltpu.VMEM((F, D), jnp.bfloat16), pltpu.VMEM((F, D), jnp.bfloat16),
                        pltpu.SemaphoreType.DMA((4,))],
        compiler_params=pltpu.CompilerParams(dimension_semantics=("arbitrary",), vmem_limit_bytes=100 * 1024 * 1024),
    )(x, A_wqkv, A_wo, B_w1.T, B_w3.T, B_w2)
    return out.reshape(1, S, D)
```
